```python
import os as _os
_os.environ.setdefault('JAX_PLATFORMS', 'cpu')
import jax
import jax.numpy as jnp

def _softmax(x, axis=-1):
    return jax.nn.softmax(x, axis=axis)

def _gelu(x):
    return jax.nn.gelu(x, approximate=True)

def _silu(x):
    return jax.nn.silu(x)

def _sigmoid(x):
    return jax.nn.sigmoid(x)

def _layernorm(x, axis=-1, eps=1e-05):
    m = jnp.mean(x, axis=axis, keepdims=True)
    v = jnp.var(x, axis=axis, keepdims=True)
    return (x - m) / jnp.sqrt(v + eps)

def _scatter_add(tgt, idx, src, axis=0):
    return tgt.at[idx].add(src)

def _segment_sum(src, seg, n):
    return jax.ops.segment_sum(src, seg, n)

class _Rng:

    def __init__(self, key):
        self._k = key

    def _next(self):
        self._k, sub = jax.random.split(self._k)
        return sub

    def normal(self, shape):
        return jax.random.normal(self._next(), shape, dtype=jnp.bfloat16)

    def randint(self, lo, hi, shape):
        return jax.random.randint(self._next(), shape, lo, hi, dtype=jnp.int32)

    def uniform(self, shape, lo=0.0, hi=1.0):
        return jax.random.uniform(self._next(), shape, jnp.bfloat16, lo, hi)

    def permutation(self, n):
        return jax.random.permutation(self._next(), n)
kernel_name = 'sequential_preLN__memory_aug_recurrent_mem_tr__swiglu_ffn__prompt'

def setup_inputs():
    _rng = _Rng(jax.random.key(int.from_bytes(__import__("os").urandom(4), "little")))
    _w = lambda a: (lambda t: t.astype(jnp.bfloat16) if jnp.issubdtype(t.dtype, jnp.floating) else t)(jnp.asarray(a))

    def _A_setup():
        B, S, Dm = (1, 2048, 640)
        H, Dh = (32, 192)
        M, seg = (8, 32)
        seg = min(seg, S)
        S = S // seg * seg
        return {'x': _w((lambda *s: _rng.normal(s) * 0.05)(B, S, Dm)), 'mem0': _w((lambda *s: _rng.normal(s) * 0.1)(B, M, Dm)), 'Wq': _w((lambda *s: _rng.normal(s) * 1.6)(Dm, H, Dh) * Dm ** (-0.5)), 'Wk': _w((lambda *s: _rng.normal(s) * 1.6)(Dm, H, Dh) * Dm ** (-0.5)), 'Wv': _w((lambda *s: _rng.normal(s) * 0.1)(Dm, H, Dh) * Dm ** (-0.5)), 'Wo': _w((lambda *s: _rng.normal(s) * 0.1)(H, Dh, Dm) * (H * Dh) ** (-0.5)), 'seg_len': seg}
    _A_in = _A_setup()

    def _B_setup():
        B, S, D, F = (1, 2048, 640, 1536)
        return {'x': _w((lambda *s: _rng.normal(s) * 0.05)(B, S, D)), 'w_gate': _w((lambda *s: _rng.normal(s) * 0.05)(D, F)), 'w_up': _w((lambda *s: _rng.normal(s) * 0.05)(D, F)), 'w_down': _w((lambda *s: _rng.normal(s) * 0.05)(F, D))}
    _B_in = _B_setup()
    return {'A_x': _A_in['x'], 'A_mem0': _A_in['mem0'], 'A_Wq': _A_in['Wq'], 'A_Wk': _A_in['Wk'], 'A_Wv': _A_in['Wv'], 'A_Wo': _A_in['Wo'], 'A_seg_len': _A_in['seg_len'], 'B_x': _B_in['x'], 'B_w_gate': _B_in['w_gate'], 'B_w_up': _B_in['w_up'], 'B_w_down': _B_in['w_down']}

def reference(A_x, A_mem0, A_Wq, A_Wk, A_Wv, A_Wo, A_seg_len, B_x, B_w_gate, B_w_up, B_w_down):

    def _A_ref(x, mem0, Wq, Wk, Wv, Wo, seg_len):
        B, S, Dm = x.shape
        H, Dh = (Wq.shape[1], Wq.shape[2])
        M = mem0.shape[1]
        scale = Dh ** (-0.5)
        n_seg = S // seg_len
        L = M + seg_len
        idx = jnp.arange(L)
        mask = (idx[:, None] < M) | (idx[:, None] >= idx[None, :])
        mem = mem0
        outs = []
        for s in range(n_seg):
            xs = x[:, s * seg_len:(s + 1) * seg_len, :].copy()
            h = jnp.concatenate([mem, xs], axis=1)
            q = jnp.einsum('btd,dhe->bhte', h, Wq)
            k = jnp.einsum('btd,dhe->bhte', h, Wk)
            v = jnp.einsum('btd,dhe->bhte', h, Wv)
            scores = jnp.einsum('bhqe,bhke->bhqk', q, k) * scale
            scores = jnp.where(mask[None, None], scores, -1000000000.0)
            p = _softmax(scores, axis=-1)
            o = jnp.einsum('bhqk,bhke->bhqe', p, v)
            o = jnp.einsum('bhte,hed->btd', o, Wo)
            mem = o[:, :M, :].copy()
            outs.append(o[:, M:, :])
        return jnp.concatenate(outs, axis=1)

    def _B_ref(x, w_gate, w_up, w_down):
        g = _silu(x @ w_gate)
        u = x @ w_up
        return g * u @ w_down
    x = A_x
    h = x + _A_ref(_layernorm(x, axis=-1), A_mem0, A_Wq, A_Wk, A_Wv, A_Wo, A_seg_len)
    h2 = h + _B_ref(_layernorm(h, axis=-1), B_w_gate, B_w_up, B_w_down)
    return h2
```

```python
import functools
import jax
import jax.numpy as jnp
from jax import lax
import jax.experimental.pallas as pl
import jax.experimental.pallas.tpu as pltpu

F32 = jnp.float32
BF16 = jnp.bfloat16
U32 = jnp.uint32
LANE = 128
NT = (((1,), (1,)), ((), ()))


def _ln(x, eps=1e-5):
    m = jnp.mean(x, axis=-1, keepdims=True)
    xc = x - m
    v = jnp.mean(xc * xc, axis=-1, keepdims=True)
    return xc * lax.rsqrt(v + eps)


def _make_kernel(S, D, H, Dh, M, SEG, FF):
    NSEG = S // SEG
    L = M + SEG
    RA = SEG - M
    RB = SEG - RA
    HD = H * Dh
    PW = 2 * Dh
    NP = H // 2
    TPP = PW // LANE
    KD = D // LANE
    NF = FF // LANE
    CH = 2 * PW
    NCH = HD // CH
    TPC = CH // LANE
    NSLOT = 4
    PF = NSLOT - 1
    SPI = NSEG // (2 * NCH)
    scale = Dh ** -0.5
    assert M == 8 and SEG == 32 and NSEG % 2 == 0 and PW % LANE == 0 and D % LANE == 0

    def kernel(x_hbm, mem0_hbm, wqt_hbm, wkt_hbm, wvt_hbm, wo_hbm, wg_hbm, wu_hbm, wd_hbm,
               out_hbm,
               x_v, xbs_v, xb_v, xa_v, mem0_v, mem_v, stage_v, wqkv_v, qkvb_v, wo_v, wg_v, wu_v, wd_v,
               h_v, out_v, sem_s, sem_m, sem_o, sem_g, sem_u, sem_d, osem):
        wts = (wqt_hbm, wkt_hbm, wvt_hbm)

        def chunk_copy(i, c, slot):
            return pltpu.make_async_copy(
                wts[i].at[pl.ds(pl.multiple_of(c * CH, CH), CH), :], stage_v.at[slot], sem_s.at[slot])

        def strip_copy(src, dst, sem, n):
            return pltpu.make_async_copy(
                src.at[:, pl.ds(pl.multiple_of(n * LANE, LANE), LANE)], dst.at[n], sem.at[n])

        c_xb = pltpu.make_async_copy(x_hbm.at[:, pl.ds(RA, RB), :], xbs_v, sem_m.at[0])
        c_m0 = pltpu.make_async_copy(mem0_hbm, mem0_v, sem_m.at[1])
        c_x = pltpu.make_async_copy(x_hbm, x_v, sem_m.at[2])
        c_xb.start()
        c_m0.start()
        for g in range(PF):
            chunk_copy(0, g, g).start()
        c_x.start()

        c_xb.wait()
        for c in range(4):
            n = NSEG // 4
            xs = xbs_v[c * n:(c + 1) * n].astype(F32).reshape(n * RB, D)
            xb_v[c * n * RB:(c + 1) * n * RB, :] = _ln(xs).astype(BF16)
        c_m0.wait()
        mem_v[...] = mem0_v[...].astype(F32)
        h_v[...] = jnp.zeros(h_v.shape, F32)

        for i in range(3):
            if i == 1:
                c_x.wait()

            def bulk_body(c, carry, i=i):
                g = i * NCH + c
                slot = g % NSLOT
                nslot = (g + PF) % NSLOT
                chunk_copy(i, c, slot).wait()

                @pl.when(c + PF < NCH)
                def _():
                    chunk_copy(i, c + PF, nslot).start()
                if i + 1 < 3:
                    @pl.when(c + PF >= NCH)
                    def _():
                        chunk_copy(i + 1, c + PF - NCH, nslot).start()
                if i == 1:
                    @pl.when(c < KD)
                    def _():
                        strip_copy(wo_hbm, wo_v, sem_o, c).start()
                        strip_copy(wd_hbm, wd_v, sem_d, c).start()
                if i == 2:
                    @pl.when(c < NF // 2)
                    def _():
                        strip_copy(wg_hbm, wg_v, sem_g, 2 * c).start()
                        strip_copy(wg_hbm, wg_v, sem_g, 2 * c + 1).start()
                        strip_copy(wu_hbm, wu_v, sem_u, 2 * c).start()
                        strip_copy(wu_hbm, wu_v, sem_u, 2 * c + 1).start()

                xb = xb_v[...]
                for t in range(TPC):
                    wt = stage_v[slot, t * LANE:(t + 1) * LANE, :]
                    y = lax.dot_general(xb, wt, NT, preferred_element_type=F32)
                    qkvb_v[g, :, t * LANE:(t + 1) * LANE] = y.astype(BF16)
                    wqkv_v[g * TPC + t] = pltpu.bitcast(wt.T, U32)
                if i >= 1:
                    s0 = ((i - 1) * NCH + c) * SPI
                    xs = x_v[pl.ds(s0, SPI), 0:RA, :].astype(F32).reshape(SPI * RA, D)
                    xa_v[pl.ds(s0, SPI)] = _ln(xs).reshape(SPI, RA, D)
                return carry
            lax.fori_loop(0, NCH, bulk_body, 0)

        for n in range(KD):
            strip_copy(wo_hbm, wo_v, sem_o, n).wait()
            strip_copy(wd_hbm, wd_v, sem_d, n).wait()
        for n in range(NF):
            strip_copy(wg_hbm, wg_v, sem_g, n).wait()
            strip_copy(wu_hbm, wu_v, sem_u, n).wait()

        def ffn_gu(hn, n0, n1):
            acts = []
            for n in range(n0, n1):
                g = jnp.dot(hn, wg_v[n], preferred_element_type=F32)
                u = jnp.dot(hn, wu_v[n], preferred_element_type=F32)
                acts.append((g * jax.nn.sigmoid(g) * u).astype(BF16))
            return acts

        def ffn_down(h, acts):
            outs = [None] * KD
            for k in range(NF):
                for n in range(KD):
                    y = jnp.dot(acts[k], wd_v[n, k * LANE:(k + 1) * LANE, :], preferred_element_type=F32)
                    outs[n] = y if outs[n] is None else outs[n] + y
            return (h + jnp.concatenate(outs, axis=1)).astype(BF16)

        def substep(s, mem, h_prev, left):
            row = lax.broadcasted_iota(jnp.int32, (L, 2 * L), 0)
            col = lax.broadcasted_iota(jnp.int32, (L, 2 * L), 1)
            is_a = col < L
            key = jnp.where(is_a, col, col - L)
            allowed = (row < M) | (row >= key)
            lane_a = lax.broadcasted_iota(jnp.int32, (L, PW), 1) < Dh

            hn = _ln(h_prev).astype(BF16)
            lhs = jnp.concatenate([mem, xa_v[s]], axis=0).astype(BF16)
            r0 = pl.multiple_of(s * RB, RB)
            acc = [None] * KD
            new_left = []

            def proj(p, i):
                j0 = i * (HD // LANE) + p * TPP
                a = jnp.concatenate(
                    [jnp.dot(lhs, pltpu.bitcast(wqkv_v[j0 + t], BF16), preferred_element_type=F32)
                     for t in range(TPP)], axis=1)
                b = qkvb_v[i * NCH + p // 2, pl.ds(r0, RB), (p % 2) * PW:(p % 2 + 1) * PW].astype(F32)
                return jnp.concatenate([a, b], axis=0)

            def bd(a):
                return jnp.concatenate([jnp.where(lane_a, a, 0.0), jnp.where(lane_a, 0.0, a)], axis=0).astype(BF16)

            def scores(q, kbd):
                sc = lax.dot_general(q, kbd, NT, preferred_element_type=F32) * scale
                sc = jnp.where(allowed, sc, -1e9)
                m_a = jnp.max(jnp.where(is_a, sc, -jnp.inf), axis=1, keepdims=True)
                m_b = jnp.max(jnp.where(is_a, -jnp.inf, sc), axis=1, keepdims=True)
                e = jnp.exp(sc - jnp.where(is_a, m_a, m_b))
                s_a = jnp.sum(jnp.where(is_a, e, 0.0), axis=1, keepdims=True)
                s_b = jnp.sum(jnp.where(is_a, 0.0, e), axis=1, keepdims=True)
                return (e * jnp.where(is_a, 1.0 / s_a, 1.0 / s_b)).astype(BF16)

            def pv(p):
                o = jnp.dot(PR.pop(p), VB.pop(p), preferred_element_type=F32)
                if left is None:
                    new_left.append(o[M + RA:])
                    O[p] = o[:M + RA].astype(BF16)
                else:
                    O[p] = jnp.concatenate([o, left[p]], axis=0).astype(BF16)

            def wo(p):
                o = O.pop(p)
                for n in range(KD):
                    y = jnp.dot(o, wo_v[n, p * PW:(p + 1) * PW, :], preferred_element_type=F32)
                    acc[n] = y if acc[n] is None else acc[n] + y

            PR, VB, O = {}, {}, {}
            for p in range(NP):
                q = proj(p, 0).astype(BF16)
                kbd = bd(proj(p, 1))
                if p >= 2:
                    pv(p - 2)
                VB[p] = bd(proj(p, 2))
                if p >= 3:
                    wo(p - 3)
                PR[p] = scores(q, kbd)
            wo(NP - 3)
            pv(NP - 2)
            acts = ffn_gu(hn, 0, NF // 2)
            wo(NP - 2)
            pv(NP - 1)
            acts += ffn_gu(hn, NF // 2, NF)
            wo(NP - 1)
            y = ffn_down(h_prev, acts)
            return jnp.concatenate(acc, axis=1), new_left, y

        def loop_body(t, carry):
            a = 2 * t
            b = a + 1
            h0 = h_v[0:SEG, :]
            h1 = h_v[SEG:2 * SEG, :]
            att_a, left, y0 = substep(a, mem_v[...], h0, None)
            att_b, _, y1 = substep(b, att_a[:M], h1, left)
            mem_v[...] = att_b[:M]
            xa = x_v[a].astype(F32)
            xb = x_v[b].astype(F32)
            h_v[0:RA, :] = xa[:RA] + att_a[M:]
            h_v[RA:SEG, :] = xa[RA:] + att_b[L:]
            h_v[SEG:2 * SEG, :] = xb + att_b[M:L]
            tp = jnp.maximum(t - 1, 0)
            out_v[tp, 0:SEG, :] = y0
            out_v[tp, SEG:2 * SEG, :] = y1

            @pl.when(t > 0)
            def _():
                pltpu.make_async_copy(out_v.at[tp], out_hbm.at[tp], osem).start()
            return carry
        lax.fori_loop(0, NSEG // 2, loop_body, 0)

        h_last = h_v[...]
        acts = ffn_gu(_ln(h_last).astype(BF16), 0, NF)
        out_v[NSEG // 2 - 1] = ffn_down(h_last, acts)
        pltpu.make_async_copy(out_v.at[NSEG // 2 - 1], out_hbm.at[NSEG // 2 - 1], osem).start()
        pltpu.make_async_copy(out_v, out_hbm, osem).wait()

    scratch = [
        pltpu.VMEM((NSEG, SEG, D), BF16),
        pltpu.VMEM((NSEG, RB, D), BF16),
        pltpu.VMEM((NSEG * RB, D), BF16),
        pltpu.VMEM((NSEG, RA, D), F32),
        pltpu.VMEM((M, D), BF16),
        pltpu.VMEM((M, D), F32),
        pltpu.VMEM((NSLOT, CH, D), BF16),
        pltpu.VMEM((3 * HD // LANE, D // 2, LANE), U32),
        pltpu.VMEM((3 * NCH, NSEG * RB, CH), BF16),
        pltpu.VMEM((KD, HD, LANE), BF16),
        pltpu.VMEM((NF, D, LANE), BF16),
        pltpu.VMEM((NF, D, LANE), BF16),
        pltpu.VMEM((KD, FF, LANE), BF16),
        pltpu.VMEM((2 * SEG, D), F32),
        pltpu.VMEM((NSEG // 2, 2 * SEG, D), BF16),
        pltpu.SemaphoreType.DMA((NSLOT,)),
        pltpu.SemaphoreType.DMA((3,)),
        pltpu.SemaphoreType.DMA((KD,)),
        pltpu.SemaphoreType.DMA((NF,)),
        pltpu.SemaphoreType.DMA((NF,)),
        pltpu.SemaphoreType.DMA((KD,)),
        pltpu.SemaphoreType.DMA(()),
    ]
    return kernel, scratch


@functools.partial(jax.jit, static_argnames=("A_seg_len",))
def pallas_sequential_preLN__memory_aug_recurrent_mem_tr__swiglu_ffn__prompt_kernel(A_x, A_mem0, A_Wq, A_Wk, A_Wv, A_Wo, A_seg_len, B_x, B_w_gate, B_w_up, B_w_down):
    B, S, D = A_x.shape
    _, H, Dh = A_Wq.shape
    M = A_mem0.shape[1]
    FF = B_w_gate.shape[1]
    SEG = A_seg_len
    assert B == 1
    kernel, scratch = _make_kernel(S, D, H, Dh, M, SEG, FF)
    tr = lambda w: w.transpose(1, 2, 0).reshape(H * Dh, D)
    out = pl.pallas_call(
        kernel,
        out_shape=jax.ShapeDtypeStruct((S // (2 * SEG), 2 * SEG, D), A_x.dtype),
        in_specs=[pl.BlockSpec(memory_space=pl.ANY)] * 9,
        out_specs=pl.BlockSpec(memory_space=pl.ANY),
        scratch_shapes=scratch,
        compiler_params=pltpu.CompilerParams(vmem_limit_bytes=110 * 1024 * 1024),
    )(A_x.reshape(S // SEG, SEG, D), A_mem0.reshape(M, D), tr(A_Wq), tr(A_Wk), tr(A_Wv),
      A_Wo.reshape(H * Dh, D), B_w_gate, B_w_up, B_w_down)
    return out.reshape(B, S, D)
```

```python
import functools
import jax
import jax.numpy as jnp
from jax import lax
import jax.experimental.pallas as pl
import jax.experimental.pallas.tpu as pltpu

F32 = jnp.float32
BF16 = jnp.bfloat16
U32 = jnp.uint32
LANE = 128
NA = 7
NB = 1
ORDER = 'QFKSVPW'
UNROLL = 2
NT = (((1,), (1,)), ((), ()))


def _ln(x, eps=1e-5):
    m = jnp.mean(x, axis=-1, keepdims=True)
    xc = x - m
    v = jnp.mean(xc * xc, axis=-1, keepdims=True)
    return xc * lax.rsqrt(v + eps)


def _make_kernel(S, D, H, Dh, M, SEG, FF):
    NSEG = S // SEG
    L = M + SEG
    RA = SEG - M
    RB = SEG - RA
    HD = H * Dh
    PW = 2 * Dh
    NP = H // 2
    TPP = PW // LANE
    KD = D // LANE
    NF = FF // LANE
    CH = 8 * LANE
    NCH = HD // CH
    TPC = CH // LANE
    NSLOT = 4
    PF = NSLOT - 1
    SPI = -(-NSEG // (2 * NCH))
    scale = Dh ** -0.5
    assert NCH == KD + 1 and NCH * 2 >= NF and TPP == 3 and M == 8 and SEG == 32 and NSEG % 2 == 0 and PW % LANE == 0 and D % LANE == 0

    def kernel(x_hbm, mem0_hbm, wqt_hbm, wkt_hbm, wvt_hbm, wo_hbm, wg_hbm, wu_hbm, wd_hbm,
               out_hbm,
               x_v, xbs_v, xb_v, xa_v, mem0_v, mem_v, stage_v, wqkv_v, qkvb_v, wo_v, wo32_v, wg_v, wu_v, wd_v,
               h_v, hn_v, out_v, sem_s, sem_m, sem_o, sem_g, sem_u, sem_d, osem):
        wts = (wqt_hbm, wkt_hbm, wvt_hbm)

        def chunk_copy(i, c, slot):
            return pltpu.make_async_copy(
                wts[i].at[pl.ds(pl.multiple_of(c * CH, CH), CH), :], stage_v.at[slot], sem_s.at[slot])

        def strip_copy(src, dst, sem, n):
            return pltpu.make_async_copy(
                src.at[:, pl.ds(pl.multiple_of(n * LANE, LANE), LANE)], dst.at[n], sem.at[n])

        c_xb = pltpu.make_async_copy(x_hbm.at[:, pl.ds(RA, RB), :], xbs_v, sem_m.at[0])
        c_m0 = pltpu.make_async_copy(mem0_hbm, mem0_v, sem_m.at[1])
        c_x = pltpu.make_async_copy(x_hbm, x_v, sem_m.at[2])
        c_xb.start()
        chunk_copy(0, 0, 0).start()
        c_m0.start()
        c_xb.wait()
        for g in range(1, PF):
            chunk_copy(0, g, g).start()
        for c in range(4):
            n = NSEG // 4
            xs = xbs_v[c * n:(c + 1) * n].astype(F32).reshape(n * RB, D)
            xb_v[c * n * RB:(c + 1) * n * RB, :] = _ln(xs).astype(BF16)
        c_m0.wait()
        mem_v[...] = mem0_v[...].astype(F32)
        h_v[...] = jnp.zeros(h_v.shape, F32)
        hn_v[...] = jnp.zeros(hn_v.shape, BF16)

        for i in range(3):
            if i == 1:
                c_x.wait()
            if i == 2:
                for n in range(KD):
                    strip_copy(wo_hbm, wo_v, sem_o, n).wait()

            def bulk_body(c, carry, i=i):
                g = i * NCH + c
                slot = g % NSLOT
                nslot = (g + PF) % NSLOT
                chunk_copy(i, c, slot).wait()

                @pl.when(c + PF < NCH)
                def _():
                    chunk_copy(i, c + PF, nslot).start()
                if i + 1 < 3:
                    @pl.when(c + PF >= NCH)
                    def _():
                        chunk_copy(i + 1, c + PF - NCH, nslot).start()
                if i == 0:
                    @pl.when(c == 0)
                    def _():
                        c_x.start()

                    @pl.when(c >= 1)
                    def _():
                        strip_copy(wo_hbm, wo_v, sem_o, c - 1).start()
                if i == 1:
                    @pl.when(c < KD)
                    def _():
                        strip_copy(wd_hbm, wd_v, sem_d, c).start()

                    @pl.when(c < NF // 2)
                    def _():
                        strip_copy(wg_hbm, wg_v, sem_g, 2 * c).start()
                        strip_copy(wg_hbm, wg_v, sem_g, 2 * c + 1).start()
                        strip_copy(wu_hbm, wu_v, sem_u, 2 * c).start()
                        strip_copy(wu_hbm, wu_v, sem_u, 2 * c + 1).start()

                xb = xb_v[...]
                for t in range(TPC):
                    wt = stage_v[slot, t * LANE:(t + 1) * LANE, :]
                    y = lax.dot_general(xb, wt, NT, preferred_element_type=F32)
                    qkvb_v[g * TPC + t] = y.astype(BF16)
                    wqkv_v[g * TPC + t] = pltpu.bitcast(wt.T, U32)
                if i >= 1:
                    s0 = jnp.minimum(((i - 1) * NCH + c) * SPI, NSEG - SPI)
                    xs = x_v[pl.ds(s0, SPI), 0:RA, :].astype(F32).reshape(SPI * RA, D)
                    xa_v[pl.ds(s0, SPI)] = _ln(xs).reshape(SPI, RA, D)
                if i == 2:
                    for n in range(KD):
                        w = wo_v[n, pl.ds(pl.multiple_of(c * CH, CH), CH), :]
                        wo32_v[n, pl.ds(pl.multiple_of(c * (CH // 2), CH // 2), CH // 2), :] = pltpu.bitcast(w, U32)
                return carry
            lax.fori_loop(0, NCH, bulk_body, 0)

        for n in range(KD):
            strip_copy(wd_hbm, wd_v, sem_d, n).wait()
        for n in range(NF):
            strip_copy(wg_hbm, wg_v, sem_g, n).wait()
            strip_copy(wu_hbm, wu_v, sem_u, n).wait()

        def ffn_gu(hn, n0, n1):
            acts = []
            for n in range(n0, n1):
                g = jnp.dot(hn, wg_v[n], preferred_element_type=F32)
                u = jnp.dot(hn, wu_v[n], preferred_element_type=F32)
                acts.append((g * jax.nn.sigmoid(g) * u).astype(BF16))
            return acts

        def ffn_down_part(outs, acts, k0, k1):
            for k in range(k0, k1):
                for n in range(KD):
                    y = jnp.dot(acts[k], wd_v[n, k * LANE:(k + 1) * LANE, :], preferred_element_type=F32)
                    outs[n] = y if outs[n] is None else outs[n] + y

        def ffn_down(h, acts):
            outs = [None] * KD
            ffn_down_part(outs, acts, 0, NF)
            return (h + jnp.concatenate(outs, axis=1)).astype(BF16)

        def substep(s, mem, left, fill, inloop):
            row = lax.broadcasted_iota(jnp.int32, (L, 2 * L), 0)
            col = lax.broadcasted_iota(jnp.int32, (L, 2 * L), 1)
            is_a = col < L
            key = jnp.where(is_a, col, col - L)
            allowed = (row < M) | (row >= key)
            lane_lo = lax.broadcasted_iota(jnp.int32, (L, LANE), 1) < Dh - LANE

            lhs = jnp.concatenate([mem, xa_v[s]], axis=0).astype(BF16)
            r0 = pl.multiple_of(s * RB, RB)
            acc = [None] * KD
            new_left = []

            def proj(p, i):
                j0 = i * (HD // LANE) + p * TPP
                tiles = []
                for t in range(TPP):
                    a = jnp.dot(lhs, pltpu.bitcast(wqkv_v[j0 + t], BF16), preferred_element_type=F32)
                    b = qkvb_v[j0 + t, pl.ds(r0, RB), :].astype(F32)
                    tiles.append(jnp.concatenate([a, b], axis=0))
                return tiles

            def stack(a, b):
                return jnp.concatenate([a, b], axis=0).astype(BF16)

            def kv_weights(t):
                return stack(t[0], t[2]), stack(jnp.where(lane_lo, t[1], 0.0), jnp.where(lane_lo, 0.0, t[1]))

            def scores(q02, q1, k02, k1):
                r02 = lax.dot_general(q02, k02, NT, preferred_element_type=F32)
                r1 = lax.dot_general(q1, k1, NT, preferred_element_type=F32)
                sc = (jnp.where(is_a, r02[:L], r02[L:]) + r1) * scale
                sc = jnp.where(allowed, sc, -1e9)
                m_a = jnp.max(jnp.where(is_a, sc, -jnp.inf), axis=1, keepdims=True)
                m_b = jnp.max(jnp.where(is_a, -jnp.inf, sc), axis=1, keepdims=True)
                e = jnp.exp(sc - jnp.where(is_a, m_a, m_b))
                e_a = jnp.where(is_a, e, 0.0)
                e_b = jnp.where(is_a, 0.0, e)
                p_a = e_a * (1.0 / jnp.sum(e_a, axis=1, keepdims=True))
                p_b = e_b * (1.0 / jnp.sum(e_b, axis=1, keepdims=True))
                return stack(p_a, p_b), (p_a + p_b).astype(BF16)

            def pv(p):
                p02, p1 = PR.pop(p)
                v02, v1 = VB.pop(p)
                o02 = jnp.dot(p02, v02, preferred_element_type=F32)
                o1 = jnp.dot(p1, v1, preferred_element_type=F32)
                o = jnp.concatenate([o02[:L], o1, o02[L:]], axis=1)
                if left is None:
                    new_left.append(o[M + RA:])
                    O[p] = o[:M + RA].astype(BF16)
                else:
                    O[p] = jnp.concatenate([o, left[p]], axis=0).astype(BF16)

            def wo(p):
                o = O.pop(p)
                for n in range(KD):
                    w = pltpu.bitcast(wo32_v[n, p * (PW // 2):(p + 1) * (PW // 2), :], BF16)
                    y = jnp.dot(o, w, preferred_element_type=F32)
                    acc[n] = y if acc[n] is None else acc[n] + y

            PR, VB, O, QK = {}, {}, {}, {}

            def sc(p):
                PR[p] = scores(*QK.pop(p))

            QQ = {}

            def op(name, p):
                if name == 'Q':
                    q = proj(p, 0)
                    QQ[p] = (stack(q[0], q[2]), q[1].astype(BF16))
                elif name == 'K':
                    QK[p] = QQ.pop(p) + kv_weights(proj(p, 1))
                elif name == 'V':
                    VB[p] = kv_weights(proj(p, 2))
                elif name == 'S':
                    if p >= 1:
                        sc(p - 1)
                elif name == 'P':
                    if p >= 2:
                        pv(p - 2)
                elif name == 'F':
                    if p in inloop:
                        inloop[p]()
                elif name == 'W':
                    if p >= 3:
                        wo(p - 3)

            for p in range(NP):
                for name in ORDER:
                    op(name, p)
            sc(NP - 1)
            wo(NP - 3)
            fill[0]()
            pv(NP - 2)
            pv(NP - 1)
            fill[1]()
            wo(NP - 2)
            wo(NP - 1)
            fill[2]()
            return jnp.concatenate(acc, axis=1), new_left

        def loop_body(t, carry):
            a = 2 * t
            b = a + 1
            h_prev = h_v[...]
            hn = hn_v[...]
            acts = {}
            gates = {}
            outs = [None] * KD

            def gate(n):
                def f():
                    gates[n] = jnp.dot(hn, wg_v[n], preferred_element_type=F32)
                return f

            def up(n):
                def f():
                    g = gates.pop(n)
                    u = jnp.dot(hn, wu_v[n], preferred_element_type=F32)
                    acts[n] = (g * jax.nn.sigmoid(g) * u).astype(BF16)
                return f

            def gu(n0, n1):
                def f():
                    for n in range(n0, n1):
                        gate(n)()
                        up(n)()
                return f

            def down(k0, k1):
                return lambda: ffn_down_part(outs, acts, k0, k1)

            in_a = {}
            for j in range(NA):
                in_a[2 + 2 * j] = gate(j)
                in_a[3 + 2 * j] = up(j)
            in_b = {1 + j: down(j, j + 1) for j in range(NB)}
            att_a, left = substep(a, mem_v[...], None, [gu(NA, NA + 3), gu(NA + 3, NA + 4), gu(NA + 4, NF)], in_a)
            att_b, _ = substep(b, att_a[:M], left, [down(NB, NB + 4), down(NB + 4, NB + 6), down(NB + 6, NF)], in_b)
            y = (h_prev + jnp.concatenate(outs, axis=1)).astype(BF16)
            mem_v[...] = att_b[:M]
            xa = x_v[a].astype(F32)
            xb = x_v[b].astype(F32)
            h_new = jnp.concatenate([xa[:RA] + att_a[M:], xa[RA:] + att_b[L:], xb + att_b[M:L]], axis=0)
            h_v[...] = h_new
            hn_v[...] = _ln(h_new).astype(BF16)
            tp = jnp.maximum(t - 1, 0)
            out_v[tp] = y

            @pl.when(t > 0)
            def _():
                pltpu.make_async_copy(out_v.at[tp], out_hbm.at[tp], osem).start()
            return carry
        lax.fori_loop(0, NSEG // 2, loop_body, 0, unroll=UNROLL)

        h_last = h_v[...]
        acts = ffn_gu(hn_v[...], 0, NF)
        out_v[NSEG // 2 - 1] = ffn_down(h_last, acts)
        pltpu.make_async_copy(out_v.at[NSEG // 2 - 1], out_hbm.at[NSEG // 2 - 1], osem).start()
        pltpu.make_async_copy(out_v, out_hbm, osem).wait()

    scratch = [
        pltpu.VMEM((NSEG, SEG, D), BF16),
        pltpu.VMEM((NSEG, RB, D), BF16),
        pltpu.VMEM((NSEG * RB, D), BF16),
        pltpu.VMEM((NSEG, RA, D), F32),
        pltpu.VMEM((M, D), BF16),
        pltpu.VMEM((M, D), F32),
        pltpu.VMEM((NSLOT, CH, D), BF16),
        pltpu.VMEM((3 * HD // LANE, D // 2, LANE), U32),
        pltpu.VMEM((3 * HD // LANE, NSEG * RB, LANE), BF16),
        pltpu.VMEM((KD, HD, LANE), BF16),
        pltpu.VMEM((KD, HD // 2, LANE), U32),
        pltpu.VMEM((NF, D, LANE), BF16),
        pltpu.VMEM((NF, D, LANE), BF16),
        pltpu.VMEM((KD, FF, LANE), BF16),
        pltpu.VMEM((2 * SEG, D), F32),
        pltpu.VMEM((2 * SEG, D), BF16),
        pltpu.VMEM((NSEG // 2, 2 * SEG, D), BF16),
        pltpu.SemaphoreType.DMA((NSLOT,)),
        pltpu.SemaphoreType.DMA((3,)),
        pltpu.SemaphoreType.DMA((KD,)),
        pltpu.SemaphoreType.DMA((NF,)),
        pltpu.SemaphoreType.DMA((NF,)),
        pltpu.SemaphoreType.DMA((KD,)),
        pltpu.SemaphoreType.DMA(()),
    ]
    return kernel, scratch


@functools.partial(jax.jit, static_argnames=("A_seg_len",))
def pallas_sequential_preLN__memory_aug_recurrent_mem_tr__swiglu_ffn__prompt_kernel(A_x, A_mem0, A_Wq, A_Wk, A_Wv, A_Wo, A_seg_len, B_x, B_w_gate, B_w_up, B_w_down):
    B, S, D = A_x.shape
    _, H, Dh = A_Wq.shape
    M = A_mem0.shape[1]
    FF = B_w_gate.shape[1]
    SEG = A_seg_len
    assert B == 1
    kernel, scratch = _make_kernel(S, D, H, Dh, M, SEG, FF)
    tr = lambda w: w.transpose(1, 2, 0).reshape(H * Dh, D)
    out = pl.pallas_call(
        kernel,
        out_shape=jax.ShapeDtypeStruct((S // (2 * SEG), 2 * SEG, D), A_x.dtype),
        in_specs=[pl.BlockSpec(memory_space=pl.ANY)] * 9,
        out_specs=pl.BlockSpec(memory_space=pl.ANY),
        scratch_shapes=scratch,
        compiler_params=pltpu.CompilerParams(vmem_limit_bytes=110 * 1024 * 1024),
    )(A_x.reshape(S // SEG, SEG, D), A_mem0.reshape(M, D), tr(A_Wq), tr(A_Wk), tr(A_Wv),
      A_Wo.reshape(H * Dh, D), B_w_gate, B_w_up, B_w_down)
    return out.reshape(B, S, D)
```

```python
import functools

import jax
import jax.numpy as jnp
from jax import lax
import jax.experimental.pallas as pl
import jax.experimental.pallas.tpu as pltpu

F32 = jnp.float32
BF16 = jnp.bfloat16
U32 = jnp.uint32
LANE = 128
NT = (((1,), (1,)), ((), ()))

UNROLL = 2
S_LAG, P_LAG, W_LAG = 2, 5, 6
FILL_A = (2, 1, 1)
FILL_B = (2, 2, 5)


def _ln(x, eps=1e-5):
    m = jnp.mean(x, axis=-1, keepdims=True)
    xc = x - m
    v = jnp.mean(xc * xc, axis=-1, keepdims=True)
    return xc * lax.rsqrt(v + eps)


def _recip(s):
    r = pl.reciprocal(s, approx=True)
    return r * (2.0 - s * r)


def _silu(g):
    return g * (0.5 * jnp.tanh(0.5 * g) + 0.5)


def _dot(a, b):
    return jnp.dot(a, b, preferred_element_type=F32)


def _dot_nt(a, b):
    return lax.dot_general(a, b, NT, preferred_element_type=F32)


def _make_kernel(S, D, H, Dh, M, SEG, FF):
    NSEG = S // SEG
    NSUP = NSEG // 2
    L = M + SEG
    RA = SEG - M
    RB = SEG - RA
    HD = H * Dh
    PW = 2 * Dh
    NP = H // 2
    NC = NP // 2
    TPP = PW // LANE
    KD = D // LANE
    NF = FF // LANE
    CH = 8 * LANE
    NCH = HD // CH
    TPC = CH // LANE
    PF = 4
    SPI = -(-NSEG // NCH)
    G0, G1 = M, 2 * M
    cexp = Dh ** -0.5 * 1.4426950408889634
    NEG = -1e30
    assert (M, SEG, TPP, KD, NCH) == (8, 32, 3, 5, 6) and S % (2 * SEG * UNROLL) == 0
    assert D % LANE == 0 and PW % LANE == 0 and HD % CH == 0 and NP % 2 == 0
    assert FF % (3 * LANE) == 0 and NF // 3 <= NCH and 2 * L + 2 * G1 <= LANE

    def kernel(x_hbm, mem0_hbm, wqt_hbm, wkt_hbm, wvt_hbm, wo_hbm, wg_hbm, wu_hbm, wd_hbm,
               out_hbm,
               x_v, xbs_v, xb_v, xa_v, mem0_v, mem_v, stage_v, wqkv_v, qkvb_v, wo_v, wg_v, wu_v, wd_v,
               h_v, hn_v, out_v, sem_s, sem_m, sem_w, osem):
        wts = (wqt_hbm, wkt_hbm, wvt_hbm)

        def chunk_copy(i, c):
            return pltpu.make_async_copy(
                wts[i].at[pl.ds(pl.multiple_of(c * CH, CH), CH), :], stage_v.at[c], sem_s.at[c])

        def strip_start(src, dst, k, n):
            pltpu.make_async_copy(
                src.at[:, pl.ds(pl.multiple_of(n * LANE, LANE), LANE)], dst.at[n], sem_w.at[k]).start()

        c_xb = pltpu.make_async_copy(x_hbm.at[:, pl.ds(RA, RB), :], xbs_v, sem_m.at[0])
        c_m0 = pltpu.make_async_copy(mem0_hbm, mem0_v, sem_m.at[1])
        c_x = pltpu.make_async_copy(x_hbm, x_v, sem_m.at[2])
        c_xb.start()
        chunk_copy(0, 0).start()
        c_m0.start()
        c_xb.wait()
        for c in range(1, PF):
            chunk_copy(0, c).start()
        for c in range(4):
            n = NSEG // 4
            xs = xbs_v[c * n:(c + 1) * n].astype(F32).reshape(n * RB, D)
            xb_v[c * n * RB:(c + 1) * n * RB, :] = _ln(xs).astype(BF16)
        c_m0.wait()
        mem_v[...] = mem0_v[...].astype(F32)
        h_v[...] = jnp.zeros(h_v.shape, F32)
        hn_v[...] = jnp.zeros(hn_v.shape, BF16)

        def bulk_chunk(g, slot, first):
            xb = xb_v[...]
            hb = xb.shape[0] // 2
            for t in range(TPC):
                wt = stage_v[slot, t * LANE:(t + 1) * LANE, :]
                w = wt.T
                if first and t == 0:
                    y = jnp.concatenate([_dot_nt(xb[:hb], wt), _dot(xb[hb:], w)], axis=0)
                else:
                    y = _dot(xb, w)
                qkvb_v[g * TPC + t] = y.astype(BF16)
                wqkv_v[g * TPC + t] = pltpu.bitcast(w, U32)

        def bulk_a(c, carry):
            chunk_copy(0, c).wait()

            @pl.when(c + PF < NCH)
            def _():
                chunk_copy(0, c + PF).start()

            @pl.when(c + PF >= NCH)
            def _():
                chunk_copy(1, c + PF - NCH).start()

            @pl.when(c == 0)
            def _():
                c_x.start()

            @pl.when(c >= 1)
            def _():
                strip_start(wo_hbm, wo_v, 0, c - 1)
            bulk_chunk(c, c, True)
            return carry
        lax.fori_loop(0, NCH, bulk_a, 0)
        c_x.wait()

        def bulk_b(j, carry):
            g0 = NCH + 2 * j
            c0 = jnp.where(j < NCH // 2, 2 * j, 2 * j - NCH)
            for u in range(2):
                chunk_copy(1, c0 + u).wait()

            @pl.when(j == 0)
            def _():
                for u in range(2):
                    chunk_copy(1, PF + u).start()

            @pl.when(jnp.logical_and(j >= 1, j <= NCH // 2))
            def _():
                for u in range(2):
                    chunk_copy(2, 2 * (j - 1) + u).start()

            @pl.when(j < NF // 3)
            def _():
                for u in range(3):
                    strip_start(wg_hbm, wg_v, 1, 3 * j + u)
                    strip_start(wu_hbm, wu_v, 2, 3 * j + u)

            @pl.when(j < KD)
            def _():
                strip_start(wd_hbm, wd_v, 3, j)

            bulk_chunk(g0, c0, True)
            s0 = jnp.minimum(j * SPI, NSEG - SPI)
            xn = _ln(x_v[pl.ds(s0, SPI)].astype(F32).reshape(SPI * SEG, D)).reshape(SPI, SEG, D)
            xa_v[pl.ds(s0, SPI)] = xn[:, :RA, :]
            xb_v[pl.ds(pl.multiple_of(s0 * RB, RB), SPI * RB), :] = (
                xn[:, RA:, :].reshape(SPI * RB, D).astype(BF16))
            bulk_chunk(g0 + 1, c0 + 1, False)
            return carry
        lax.fori_loop(0, NCH, bulk_b, 0)

        for k, buf in enumerate((wo_v, wg_v, wu_v, wd_v)):
            pltpu.make_async_copy(buf, buf, sem_w.at[k]).wait()

        def lane_lt(shape, n):
            return lax.broadcasted_iota(jnp.int32, shape, 1) < n

        def stack(*xs):
            return jnp.concatenate(xs, axis=0).astype(BF16)

        def lo(x):
            return jnp.where(lane_lt(x.shape, Dh - LANE), x, 0.0)

        def hi(x):
            return jnp.where(lane_lt(x.shape, Dh - LANE), 0.0, x)

        def pad_lanes(x):
            return jnp.concatenate([x, jnp.zeros((x.shape[0], LANE - x.shape[1]), x.dtype)], axis=1)

        def mid_weights(th, tg):
            return stack(lo(th), hi(th), lo(tg[:G1]), hi(tg[:G1])), stack(lo(tg), hi(tg))

        class Ffn:
            def __init__(self):
                self.h = h_v[...]
                self.hn = hn_v[...]
                self.g, self.a, self.out = {}, {}, [None] * KD

            def gate(self, n):
                self.g[n] = _dot(self.hn, wg_v[n])

            def up(self, n):
                self.a[n] = (_silu(self.g.pop(n)) * _dot(self.hn, wu_v[n])).astype(BF16)

            def gu(self, n0, n1):
                for n in range(n0, n1):
                    self.gate(n)
                    self.up(n)

            def down(self, k0, k1):
                for k in range(k0, k1):
                    for n in range(KD):
                        y = _dot(self.a[k], wd_v[n, k * LANE:(k + 1) * LANE, :])
                        self.out[n] = y if self.out[n] is None else self.out[n] + y

            def result(self):
                return (self.h + jnp.concatenate(self.out, axis=1)).astype(BF16)

        def substep(s, mem, left, fill, inloop):
            row = lax.broadcasted_iota(jnp.int32, (L, 2 * L), 0)
            col = lax.broadcasted_iota(jnp.int32, (L, 2 * L), 1)
            ok_a = (col < L) & ((row < M) | (row >= col))
            ok_b = (col >= L) & ((row < M) | (row >= col - L))

            lhs = stack(mem, xa_v[s])
            r0 = pl.multiple_of(s * RB, RB)
            acc = [None] * KD
            new_left = {}
            PR, O, QT, KT, VT = {}, {}, {}, {}, {}

            def proj(p, i):
                j0 = i * (HD // LANE) + p * TPP
                return [jnp.concatenate([_dot(lhs, pltpu.bitcast(wqkv_v[j0 + t], BF16)),
                                         qkvb_v[j0 + t, pl.ds(r0, RB), :].astype(F32)], axis=0)
                        for t in range(TPP)]

            def softmax(r02, r1):
                ps = []
                for r, ok in ((r02[:L], ok_a), (r02[L:], ok_b)):
                    sc = jnp.where(ok, r + r1, NEG)
                    e = jnp.exp2((sc - jnp.max(sc, axis=1, keepdims=True)) * cexp)
                    ps.append(e * _recip(jnp.sum(e, axis=1, keepdims=True)))
                return ps

            def scores(c):
                h, g = 2 * c, 2 * c + 1
                qh, qg, kh, kg = QT.pop(h), QT.pop(g), KT.pop(h), KT.pop(g)
                wx, wy = mid_weights(kh[1], kg[1])
                r02h = _dot_nt(stack(qh[0], qh[2]), stack(kh[0], kh[2]))
                r1x = _dot_nt(stack(qh[1], qg[1][G0:G1]), wx)
                r02g = _dot_nt(stack(qg[0], qg[2]), stack(kg[0], kg[2]))
                r1y = _dot_nt(stack(qg[1][:G0], qg[1][G1:]), wy)
                z = pad_lanes(r1x[L:])
                za = pltpu.roll(z, LANE - 2 * L, 1)[:, :2 * L]
                zb = pltpu.roll(z, LANE - L - G1, 1)[:, :2 * L]
                r1g = jnp.concatenate(
                    [r1y[:G0], jnp.where(lane_lt(za.shape, L), za, zb), r1y[G0:]], axis=0)
                pah, pbh = softmax(r02h, r1x[:L, :2 * L])
                pag, pbg = softmax(r02g, r1g)
                pg = pag + pbg
                zg = (pltpu.roll(pad_lanes(pag[G0:G1]), 2 * L, 1)
                      + pltpu.roll(pad_lanes(pbg[G0:G1]), L + G1, 1))[:, :2 * L + 2 * G1]
                ph = pad_lanes(pah + pbh)[:, :2 * L + 2 * G1]
                PR[c] = (stack(pah, pbh), stack(ph, zg), stack(pag, pbg), stack(pg[:G0], pg[G1:]))

            def finish(p, o):
                if left is None:
                    new_left[p] = o[M + RA:]
                    O[p] = o[:M + RA].astype(BF16)
                else:
                    O[p] = stack(o, left[p])

            def pv(c):
                h, g = 2 * c, 2 * c + 1
                p02h, p1x, p02g, p1y = PR.pop(c)
                vh, vg = VT.pop(h), VT.pop(g)
                wx, wy = mid_weights(vh[1], vg[1])
                o02h = _dot(p02h, stack(vh[0], vh[2]))
                o1x = _dot(p1x, wx)
                o02g = _dot(p02g, stack(vg[0], vg[2]))
                o1y = _dot(p1y, wy)
                o1g = jnp.concatenate([o1y[:G0], o1x[L:], o1y[G0:]], axis=0)
                finish(h, jnp.concatenate([o02h[:L], o1x[:L], o02h[L:]], axis=1))
                finish(g, jnp.concatenate([o02g[:L], o1g, o02g[L:]], axis=1))

            def wo(p):
                o = O.pop(p)
                for n in range(KD):
                    y = _dot(o, wo_v[n, p * PW:(p + 1) * PW, :])
                    acc[n] = y if acc[n] is None else acc[n] + y

            for p in range(NP):
                QT[p] = proj(p, 0)
                for f in inloop.get(p, ()):
                    f()
                KT[p] = proj(p, 1)
                if p >= S_LAG and (p - S_LAG) % 2 == 0:
                    scores((p - S_LAG) // 2)
                if p >= P_LAG and (p - P_LAG) % 2 == 0:
                    pv((p - P_LAG) // 2)
                VT[p] = proj(p, 2)
                if p >= W_LAG:
                    wo(p - W_LAG)
            scores(NC - 1)
            for p in sorted(O):
                wo(p)
            for c in sorted(PR)[:-1]:
                pv(c)
            fill[0]()
            for p in sorted(O):
                wo(p)
            pv(NC - 1)
            fill[1]()
            wo(NP - 2)
            wo(NP - 1)
            fill[2]()
            assert not (PR or O or QT or KT or VT)
            return jnp.concatenate(acc, axis=1), new_left

        def spread(ops, p0):
            slots = {}
            for i, f in enumerate(ops):
                slots.setdefault(p0 + (i * (NP - p0)) // len(ops), []).append(f)
            return slots

        def loop_body(t, carry):
            a = 2 * t
            b = a + 1
            ffn = Ffn()
            P = functools.partial
            na, nb = NF - sum(FILL_A), NF - sum(FILL_B)
            in_a = spread([P(f, n) for n in range(na) for f in (ffn.gate, ffn.up)], 1)
            in_b = spread([P(ffn.down, k, k + 1) for k in range(nb)], 0)
            a1, a2 = na + FILL_A[0], na + FILL_A[0] + FILL_A[1]
            b1, b2 = nb + FILL_B[0], nb + FILL_B[0] + FILL_B[1]
            att_a, left = substep(a, mem_v[...], None,
                                  [P(ffn.gu, na, a1), P(ffn.gu, a1, a2), P(ffn.gu, a2, NF)], in_a)
            att_b, _ = substep(b, att_a[:M], left,
                               [P(ffn.down, nb, b1), P(ffn.down, b1, b2), P(ffn.down, b2, NF)], in_b)
            y = ffn.result()
            mem_v[...] = att_b[:M]
            xa = x_v[a].astype(F32)
            xb = x_v[b].astype(F32)
            h_new = jnp.concatenate(
                [xa[:RA] + att_a[M:], xa[RA:] + att_b[L:], xb + att_b[M:L]], axis=0)
            h_v[...] = h_new
            hn_v[...] = _ln(h_new).astype(BF16)
            tp = jnp.maximum(t - 1, 0)
            out_v[tp] = y

            @pl.when(t > 0)
            def _():
                pltpu.make_async_copy(out_v.at[tp], out_hbm.at[tp], osem).start()
            return carry
        lax.fori_loop(0, NSUP, loop_body, 0, unroll=UNROLL)

        ffn = Ffn()
        ffn.gu(0, NF)
        ffn.down(0, NF)
        out_v[NSUP - 1] = ffn.result()
        pltpu.make_async_copy(out_v.at[NSUP - 1], out_hbm.at[NSUP - 1], osem).start()
        pltpu.make_async_copy(out_v, out_hbm, osem).wait()

    scratch = [
        pltpu.VMEM((NSEG, SEG, D), BF16),
        pltpu.VMEM((NSEG, RB, D), BF16),
        pltpu.VMEM((NSEG * RB, D), BF16),
        pltpu.VMEM((NSEG, RA, D), F32),
        pltpu.VMEM((M, D), BF16),
        pltpu.VMEM((M, D), F32),
        pltpu.VMEM((NCH, CH, D), BF16),
        pltpu.VMEM((3 * HD // LANE, D // 2, LANE), U32),
        pltpu.VMEM((3 * HD // LANE, NSEG * RB, LANE), BF16),
        pltpu.VMEM((KD, HD, LANE), BF16),
        pltpu.VMEM((NF, D, LANE), BF16),
        pltpu.VMEM((NF, D, LANE), BF16),
        pltpu.VMEM((KD, FF, LANE), BF16),
        pltpu.VMEM((2 * SEG, D), F32),
        pltpu.VMEM((2 * SEG, D), BF16),
        pltpu.VMEM((NSUP, 2 * SEG, D), BF16),
        pltpu.SemaphoreType.DMA((NCH,)),
        pltpu.SemaphoreType.DMA((3,)),
        pltpu.SemaphoreType.DMA((4,)),
        pltpu.SemaphoreType.DMA(()),
    ]
    return kernel, scratch


@functools.partial(jax.jit, static_argnames=("seg",))
def _run(x, mem0, wq, wk, wv, wo, wg, wu, wd, seg):
    B, S, D = x.shape
    _, H, Dh = wq.shape
    M = mem0.shape[1]
    FF = wg.shape[1]
    assert B == 1
    kernel, scratch = _make_kernel(S, D, H, Dh, M, seg, FF)
    tr = lambda w: w.transpose(1, 2, 0).reshape(H * Dh, D)
    out = pl.pallas_call(
        kernel,
        out_shape=jax.ShapeDtypeStruct((S // (2 * seg), 2 * seg, D), x.dtype),
        in_specs=[pl.BlockSpec(memory_space=pl.ANY)] * 9,
        out_specs=pl.BlockSpec(memory_space=pl.ANY),
        scratch_shapes=scratch,
        compiler_params=pltpu.CompilerParams(
            vmem_limit_bytes=100 * 1024 * 1024, disable_bounds_checks=True),
    )(x.reshape(S // seg, seg, D), mem0.reshape(M, D), tr(wq), tr(wk), tr(wv),
      wo.reshape(H * Dh, D), wg, wu, wd)
    return out.reshape(B, S, D)


def pallas_sequential_preLN__memory_aug_recurrent_mem_tr__swiglu_ffn__prompt_kernel(A_x, A_mem0, A_Wq, A_Wk, A_Wv, A_Wo, A_seg_len, B_x, B_w_gate, B_w_up, B_w_down):
    seg = A_seg_len if isinstance(A_seg_len, int) else 32
    return _run(A_x, A_mem0, A_Wq, A_Wk, A_Wv, A_Wo, B_w_gate, B_w_up, B_w_down, seg=seg)
```
